```python
import os as _os
_os.environ.setdefault("JAX_PLATFORMS", "cpu")
import jax
import jax.numpy as jnp

def _softmax(x, axis=-1):
    return jax.nn.softmax(x, axis=axis)
def _gelu(x):
    return jax.nn.gelu(x, approximate=True)
def _silu(x):
    return jax.nn.silu(x)
def _sigmoid(x):
    return jax.nn.sigmoid(x)
def _layernorm(x, axis=-1, eps=1e-5):
    m = jnp.mean(x, axis=axis, keepdims=True)
    v = jnp.var(x, axis=axis, keepdims=True)
    return (x - m) / jnp.sqrt(v + eps)
def _scatter_add(tgt, idx, src, axis=0):
    return tgt.at[idx].add(src)
def _segment_sum(src, seg, n):
    return jax.ops.segment_sum(src, seg, n)
class _Rng:
    def __init__(self, key):
        self._k = key
    def _next(self):
        self._k, sub = jax.random.split(self._k)
        return sub
    def normal(self, shape):
        return jax.random.normal(self._next(), shape, dtype=jnp.bfloat16)
    def randint(self, lo, hi, shape):
        return jax.random.randint(self._next(), shape, lo, hi, dtype=jnp.int32)
    def uniform(self, shape, lo=0.0, hi=1.0):
        return jax.random.uniform(self._next(), shape, jnp.bfloat16, lo, hi)
    def permutation(self, n):
        return jax.random.permutation(self._next(), n)


kernel_name = 'sequential_preLN__softmax_full_mha__dense_activation_gelu__prompt'

def setup_inputs():
    _rng = _Rng(jax.random.key(int.from_bytes(__import__("os").urandom(4), "little")))
    _w = (lambda a: (lambda t: t.astype(jnp.bfloat16) if jnp.issubdtype(t.dtype, jnp.floating) else t)(jnp.asarray(a)))
    def _A_setup():
        B, S, D = 1, 2048, 640
        return {
            "x": _w((lambda *s: _rng.normal(s) * 0.05)(B, S, D)),
            "wqkv": _w((lambda *s: _rng.normal(s) * 0.05)(D, 3 * D)),
            "wo": _w((lambda *s: _rng.normal(s) * 0.05)(D, D)),
        }
    _A_in = _A_setup()

    def _B_setup():
        B, S, D, F = 1, 2048, 640, 1536
        return {
            "x": _w((lambda *s: _rng.normal(s) * 0.05)(B, S, D)),
            "w1": _w((lambda *s: _rng.normal(s) * 0.4)(D, F) * (D ** -0.5)),
            "b1": _w((lambda *s: _rng.normal(s) * 0.4)(F) * 0.01),
            "w2": _w((lambda *s: _rng.normal(s) * 0.4)(F, D) * (F ** -0.5)),
            "b2": _w((lambda *s: _rng.normal(s) * 0.05)(D) * 0.01),
        }
    _B_in = _B_setup()

    return {
        "A_x": _A_in["x"],
        "A_wqkv": _A_in["wqkv"],
        "A_wo": _A_in["wo"],
        "B_x": _B_in["x"],
        "B_w1": _B_in["w1"],
        "B_b1": _B_in["b1"],
        "B_w2": _B_in["w2"],
        "B_b2": _B_in["b2"],
    }

def reference(A_x, A_wqkv, A_wo, B_x, B_w1, B_b1, B_w2, B_b2):
    def _A_ref(x, wqkv, wo):
        B, S, D = x.shape
        H = 32; Dh = D // H
        qkv = (lambda x, *d: x.transpose(*d))((x @ wqkv).reshape(B, S, 3, H, Dh), 2, 0, 3, 1, 4)
        q, k, v = qkv[0], qkv[1], qkv[2]
        scale = Dh ** -0.5
        scores = jnp.einsum("bhqd,bhkd->bhqk", q, k) * scale
        p = _softmax(scores, axis=-1)
        o = jnp.einsum("bhqk,bhkd->bhqd", p, v)
        return (lambda x, *d: x.transpose(*d))(o, 0, 2, 1, 3).reshape(B, S, D) @ wo

    def _B_ref(x, w1, b1, w2, b2):
        h = jnp.einsum("bsd,df->bsf", x, w1) + b1
        h = _gelu(h)
        return jnp.einsum("bsf,fd->bsd", h, w2) + b2

    x = A_x
    h = x + _A_ref(_layernorm(x, axis=-1), A_wqkv, A_wo)
    h2 = h + _B_ref(_layernorm(h, axis=-1), B_w1, B_b1, B_w2, B_b2)
    return h2
```

```python
import jax
import jax.numpy as jnp
from jax import lax
import jax.experimental.pallas as pl
import jax.experimental.pallas.tpu as pltpu

S, D, H, DH, HP, F = 2048, 640, 32, 20, 32, 1536
TQ = 2048
TK = 128
R = 512
NR = S // R
f32, bf16 = jnp.float32, jnp.bfloat16


def _ln(x):
    m = jnp.mean(x, axis=-1, keepdims=True)
    c = x - m
    v = jnp.mean(c * c, axis=-1, keepdims=True)
    return c * lax.rsqrt(v + 1e-5)


def _dot(a, b):
    return jnp.dot(a, b, preferred_element_type=f32)


def _kernel(x_ref, wqkv_ref, wo_hbm, w1_hbm, b1_ref, w2_hbm, b2_ref, o_ref,
            t_ref, pad_ref, q_ref, k_ref, v_ref, s_ref, op_ref,
            wo_ref, w1_ref, w2_ref, sem):
    cps = [pltpu.make_async_copy(a, b, sem.at[i]) for i, (a, b) in enumerate(
        ((wo_hbm, wo_ref), (w1_hbm, w1_ref), (w2_hbm, w2_ref)))]
    for c in cps:
        c.start()

    pad_ref[...] = jnp.zeros(pad_ref.shape, f32)
    for h in range(H):
        pad_ref[2, pl.ds(h * HP + DH, 1), :] = jnp.ones((1, R), f32)
    qscale = DH ** -0.5 * 1.4426950408889634

    def proj(r, _):
        r0 = pl.multiple_of(r * R, R)
        xn = _ln(x_ref[pl.ds(r0, R), :].astype(f32)).astype(bf16)
        qkv = _dot(xn, wqkv_ref[...])
        t_ref[...] = qkv.T
        for j in range(3):
            for h in range(H):
                blk = t_ref[pl.ds(j * D + h * DH, DH), :]
                if j == 0:
                    blk = blk * qscale
                pad_ref[j, pl.ds(h * HP, DH), :] = blk
        for g in range(H // 4):
            q_ref[g, r] = pad_ref[0, pl.ds(g * 128, 128), :]
            k_ref[g, pl.ds(r0, R), :] = pad_ref[1, pl.ds(g * 128, 128), :].T.astype(bf16)
        for h in range(H):
            v_ref[h, r] = pad_ref[2, pl.ds(h * HP, HP), :].astype(bf16)
        return 0

    lax.fori_loop(0, NR, proj, 0)

    nq = TQ // R
    nk = TK // R
    hid = lax.broadcasted_iota(jnp.int32, (128, TQ), 0) // HP

    def attn(i, _):
        h = i // (S // TQ)
        qb = i % (S // TQ)
        g = h // 4
        q = jnp.concatenate([q_ref[g, qb * nq + a] for a in range(nq)], axis=1)
        q = jnp.where(hid == h % 4, q, 0.0).astype(bf16)
        m = acc = None
        for c in range(S // TK):
            s = _dot(k_ref[g, pl.ds(c * TK, TK), :], q)
            mc = jnp.max(s.reshape(TK // 8, 8, TQ), axis=0)
            mc = jnp.max(mc, axis=0, keepdims=True)
            mn = mc if m is None else jnp.maximum(m, mc)
            p = jnp.exp2(s - mn).astype(bf16)
            if TK >= R:
                v = jnp.concatenate([v_ref[h, c * nk + a] for a in range(nk)], axis=1)
            else:
                v = v_ref[h, c * TK // R, :, pl.ds(c * TK % R, TK)]
            o = _dot(v[:24], p)
            acc = o if acc is None else acc * jnp.exp2(m - mn) + o
            m = mn
        o = acc / acc[DH:DH + 1, :]
        for a in range(nq):
            op_ref[qb * nq + a, h, :24] = o[:, a * R:(a + 1) * R]
        return 0

    lax.fori_loop(0, H * (S // TQ), attn, 0)
    for c in cps:
        c.wait()

    def ffn(r, _):
        r0 = pl.multiple_of(r * R, R)
        for h in range(H):
            t_ref[pl.ds(h * DH, DH), :] = op_ref[r, h, pl.ds(0, DH), :]
        o = t_ref[pl.ds(0, D), :].T.astype(bf16)
        hh = x_ref[pl.ds(r0, R), :].astype(f32) + _dot(o, wo_ref[...])
        u = _dot(_ln(hh).astype(bf16), w1_ref[...]) + b1_ref[...].astype(f32)
        u = jax.nn.gelu(u, approximate=True).astype(bf16)
        y = hh + _dot(u, w2_ref[...]) + b2_ref[...].astype(f32)
        o_ref[pl.ds(r0, R), :] = y.astype(o_ref.dtype)
        return 0

    lax.fori_loop(0, NR, ffn, 0)


@jax.jit
def pallas_sequential_preLN__softmax_full_mha__dense_activation_gelu__prompt_kernel(
        A_x, A_wqkv, A_wo, B_x, B_w1, B_b1, B_w2, B_b2):
    vm = pl.BlockSpec(memory_space=pltpu.VMEM)
    hb = pl.BlockSpec(memory_space=pl.ANY)
    out = pl.pallas_call(
        _kernel,
        out_shape=jax.ShapeDtypeStruct((S, D), A_x.dtype),
        in_specs=[vm, vm, hb, hb, vm, hb, vm],
        out_specs=vm,
        scratch_shapes=[
            pltpu.VMEM((3 * D, R), f32),
            pltpu.VMEM((3, H * HP, R), f32),
            pltpu.VMEM((H // 4, NR, 128, R), f32),
            pltpu.VMEM((H // 4, S, 128), bf16),
            pltpu.VMEM((H, NR, HP, R), bf16),
            pltpu.VMEM((S, TQ), f32),
            pltpu.VMEM((NR, H, HP, R), f32),
            pltpu.VMEM((D, D), bf16),
            pltpu.VMEM((D, F), bf16),
            pltpu.VMEM((F, D), bf16),
            pltpu.SemaphoreType.DMA((3,)),
        ],
        compiler_params=pltpu.CompilerParams(vmem_limit_bytes=100 * 1024 * 1024),
    )(A_x.reshape(S, D), A_wqkv, A_wo, B_w1, B_b1.reshape(1, F), B_w2, B_b2.reshape(1, D))
    return out.reshape(1, S, D)
```
